```python
import os as _os
_os.environ.setdefault('JAX_PLATFORMS', 'cpu')
import jax
import jax.numpy as jnp

def _softmax(x, axis=-1):
    return jax.nn.softmax(x, axis=axis)

def _gelu(x):
    return jax.nn.gelu(x, approximate=True)

def _silu(x):
    return jax.nn.silu(x)

def _sigmoid(x):
    return jax.nn.sigmoid(x)

def _layernorm(x, axis=-1, eps=1e-05):
    m = jnp.mean(x, axis=axis, keepdims=True)
    v = jnp.var(x, axis=axis, keepdims=True)
    return (x - m) / jnp.sqrt(v + eps)

def _scatter_add(tgt, idx, src, axis=0):
    return tgt.at[idx].add(src)

def _segment_sum(src, seg, n):
    return jax.ops.segment_sum(src, seg, n)

class _Rng:

    def __init__(self, key):
        self._k = key

    def _next(self):
        self._k, sub = jax.random.split(self._k)
        return sub

    def normal(self, shape):
        return jax.random.normal(self._next(), shape, dtype=jnp.bfloat16)

    def randint(self, lo, hi, shape):
        return jax.random.randint(self._next(), shape, lo, hi, dtype=jnp.int32)

    def uniform(self, shape, lo=0.0, hi=1.0):
        return jax.random.uniform(self._next(), shape, jnp.bfloat16, lo, hi)

    def permutation(self, n):
        return jax.random.permutation(self._next(), n)
kernel_name = 'recurrent_scan__memory_aug_recurrent_mem_tr__mixer_gmlp__prompt'

def setup_inputs():
    _rng = _Rng(jax.random.key(int.from_bytes(__import__("os").urandom(4), "little")))
    _w = lambda a: (lambda t: t.astype(jnp.bfloat16) if jnp.issubdtype(t.dtype, jnp.floating) else t)(jnp.asarray(a))

    def _A_setup():
        B, S, Dm = (1, 2048, 640)
        H, Dh = (32, 128)
        M, seg = (8, 32)
        seg = min(seg, S)
        S = S // seg * seg
        return {'x': _w((lambda *s: _rng.normal(s) * 0.05)(B, S, Dm)), 'mem0': _w((lambda *s: _rng.normal(s) * 0.1)(B, M, Dm)), 'Wq': _w((lambda *s: _rng.normal(s) * 1.6)(Dm, H, Dh) * Dm ** (-0.5)), 'Wk': _w((lambda *s: _rng.normal(s) * 1.6)(Dm, H, Dh) * Dm ** (-0.5)), 'Wv': _w((lambda *s: _rng.normal(s) * 0.1)(Dm, H, Dh) * Dm ** (-0.5)), 'Wo': _w((lambda *s: _rng.normal(s) * 0.1)(H, Dh, Dm) * (H * Dh) ** (-0.5)), 'seg_len': seg}
    _A_in = _A_setup()

    def _B_setup():
        B, S, D, F = (1, 2048, 640, 1728)
        Fh = F // 2
        return {'x': _w((lambda *s: _rng.normal(s) * 0.05)(B, S, D)), 'w_in': _w((lambda *s: _rng.normal(s) * 0.8)(D, 2 * Fh)), 'w_sp': _w(0.01 * (lambda *s: _rng.normal(s) * 0.8)(S, S)), 'b_sp': _w(1.0 + 0.01 * (lambda *s: _rng.normal(s) * 0.05)(S)), 'w_out': _w((lambda *s: _rng.normal(s) * 0.05)(Fh, D))}
    _B_in = _B_setup()
    return {'A_x': _A_in['x'], 'A_mem0': _A_in['mem0'], 'A_Wq': _A_in['Wq'], 'A_Wk': _A_in['Wk'], 'A_Wv': _A_in['Wv'], 'A_Wo': _A_in['Wo'], 'A_seg_len': _A_in['seg_len'], 'B_x': _B_in['x'], 'B_w_in': _B_in['w_in'], 'B_w_sp': _B_in['w_sp'], 'B_b_sp': _B_in['b_sp'], 'B_w_out': _B_in['w_out']}

def reference(A_x, A_mem0, A_Wq, A_Wk, A_Wv, A_Wo, A_seg_len, B_x, B_w_in, B_w_sp, B_b_sp, B_w_out):

    def _A_ref(x, mem0, Wq, Wk, Wv, Wo, seg_len):
        B, S, Dm = x.shape
        H, Dh = (Wq.shape[1], Wq.shape[2])
        M = mem0.shape[1]
        scale = Dh ** (-0.5)
        n_seg = S // seg_len
        L = M + seg_len
        idx = jnp.arange(L)
        mask = (idx[:, None] < M) | (idx[:, None] >= idx[None, :])
        mem = mem0
        outs = []
        for s in range(n_seg):
            xs = x[:, s * seg_len:(s + 1) * seg_len, :].copy()
            h = jnp.concatenate([mem, xs], axis=1)
            q = jnp.einsum('btd,dhe->bhte', h, Wq)
            k = jnp.einsum('btd,dhe->bhte', h, Wk)
            v = jnp.einsum('btd,dhe->bhte', h, Wv)
            scores = jnp.einsum('bhqe,bhke->bhqk', q, k) * scale
            scores = jnp.where(mask[None, None], scores, -1000000000.0)
            p = _softmax(scores, axis=-1)
            o = jnp.einsum('bhqk,bhke->bhqe', p, v)
            o = jnp.einsum('bhte,hed->btd', o, Wo)
            mem = o[:, :M, :].copy()
            outs.append(o[:, M:, :])
        return jnp.concatenate(outs, axis=1)

    def _B_ref(x, w_in, w_sp, b_sp, w_out):
        B, S, D = x.shape
        F = w_in.shape[-1]
        Fh = F // 2
        z = _gelu(jnp.einsum('bsd,df->bsf', x, w_in))
        z1 = z[..., :Fh].copy()
        z2 = _layernorm(z[..., Fh:], axis=-1)
        g = jnp.einsum('ts,bsf->btf', w_sp, z2) + b_sp[None, :, None]
        return jnp.einsum('bsf,fd->bsd', z1 * g, w_out)
    x = A_x
    xn = _layernorm(x, axis=-1)
    s = _A_ref(xn, A_mem0, A_Wq, A_Wk, A_Wv, A_Wo, A_seg_len)
    g = _silu(_B_ref(xn, B_w_in, B_w_sp, B_b_sp, B_w_out))
    return x + s * g
```

```python
import functools
import itertools

import jax
import jax.numpy as jnp
from jax import lax
import jax.experimental.pallas as pl
import jax.experimental.pallas.tpu as pltpu

F32 = jnp.float32
BF16 = jnp.bfloat16
U32 = jnp.uint32

LANES = 128
SUBLANES = 8
CHUNK = 144
STEP_UNROLL = 3
QK_DELAY = 2
PV_DELAY = 4
LN_EPS = 1e-5
MASK_VALUE = -1000000000.0
FLAGS = None
SKIP3 = False


def _dot(a, b):
    return jnp.dot(a, b, preferred_element_type=F32)


def _dot_nt(a, b):
    return lax.dot_general(a, b, (((1,), (1,)), ((), ())), preferred_element_type=F32)


def _as_bf16(words):
    return pltpu.bitcast(words, BF16)


def _layernorm(v):
    n = v.shape[-1]
    mean = jnp.sum(v, axis=-1, keepdims=True) * (1.0 / n)
    c = v - mean
    var = jnp.sum(c * c, axis=-1, keepdims=True) * (1.0 / n)
    return c * lax.rsqrt(var + LN_EPS)


def _gelu(v):
    inner = v * (0.7978845608028654 + (0.7978845608028654 * 0.044715) * (v * v))
    half = 0.5 * v
    return half + half * jnp.tanh(inner)


def _silu(v):
    half = 0.5 * v
    return half + half * jnp.tanh(half)


def _left_operands(a11, a12, a21, a22):
    return (a11 + a22, a21 + a22, a11, a22, a11 + a12, a21 - a11, a12 - a22)


def _right_operands(b11, b12, b21, b22):
    return (b11 + b22, b11, b12 - b22, b21 - b11, b22, b11 + b12, b21 + b22)


def _kernel(
    x_hbm, mem_hbm, wq_hbm, wk_hbm, wv_hbm, wo_hbm, win_hbm, wsp_hbm, b_hbm, wout_hbm,
    out_hbm,
    x_v, mem_v, wqkv_v, wo_v, win_v, wsp_v, b_v, wout_v,
    xn_v, xn_ops, win_ops, z1_v, z2_v, moment_v, bias_v, z2_ops, gated_v, wout_ops, wout_rest, gate_v, out_v,
    x_sem, win_sem, wsp_sem, wqkv_sem, misc_sem, out_sem,
    *, seg,
):
    S, D = x_v.shape
    M = mem_v.shape[0]
    H = wqkv_v.shape[1]
    FH = wout_v.shape[0]
    n_blocks = S // LANES
    n_pairs = n_blocks // 2
    n_seg = S // seg
    d_tiles = D // LANES
    L = M + seg

    KD = d_tiles // 2 * LANES
    KF = FH // (2 * LANES) * LANES
    half_f = FH // 2
    half_d = D // 2
    group = H // 2 // n_pairs

    def rows(i, n=1):
        start = i * LANES
        return pl.ds(start if isinstance(i, int) else pl.multiple_of(start, LANES), n * LANES)

    def x_copy(i, n, sem):
        return pltpu.make_async_copy(x_hbm.at[rows(i, n)], x_v.at[rows(i, n)], x_sem.at[sem])

    def wsp_copies(j):
        return [pltpu.make_async_copy(wsp_hbm.at[rows(i)], wsp_v.at[rows(i)], wsp_sem.at[j])
                for i in (j, j + n_pairs)]

    def wqkv_copies(g):
        return [pltpu.make_async_copy(w_hbm.bitcast(U32).at[:, par, g * group + i, :],
                                      wqkv_v.at[m, 2 * (g * group + i) + par], wqkv_sem.at[0])
                for m, w_hbm in enumerate((wq_hbm, wk_hbm, wv_hbm))
                for i in range(group) for par in range(2)]

    x_first = [x_copy(0, 1, 0), x_copy(n_pairs, 1, 0)]
    x_rest = [x_copy(1, n_pairs - 1, 1), x_copy(n_pairs + 1, n_pairs - 1, 1)]
    win_spans = [(c, CHUNK) for c in range(0, half_f, CHUNK)] + [(half_f, half_f)]
    win_cp = [[pltpu.make_async_copy(win_hbm.at[pl.ds(r + c, n)], win_v.at[pl.ds(r + c, n)],
                                     win_sem.at[i]) for r in (FH, 0)]
              for i, (c, n) in enumerate(win_spans)]
    b_cp = pltpu.make_async_copy(b_hbm, b_v, misc_sem.at[1])
    wout_cp = pltpu.make_async_copy(wout_hbm, wout_v, misc_sem.at[2])
    mem_cp = pltpu.make_async_copy(mem_hbm, mem_v, misc_sem.at[3])

    def wo_copy(n):
        return pltpu.make_async_copy(wo_hbm.at[:, rows(n)], wo_v.at[n], misc_sem.at[4])

    def start(copies):
        for cp in copies:
            cp.start()

    def wait(copies):
        for cp in copies:
            cp.wait()

    def mix_operands(j):
        xa, xb = (_layernorm(x_v[rows(i), :].astype(F32)) for i in (j, j + n_pairs))
        xn_v[rows(j), :] = xa
        xn_v[rows(j + n_pairs), :] = xb
        ops = _right_operands(xa[:, :KD], xb[:, :KD], xa[:, KD:2 * KD], xb[:, KD:2 * KD])
        ops = [op.astype(BF16) for op in ops]
        ops.append(jnp.concatenate([xa[:, 2 * KD:], xb[:, 2 * KD:]], axis=1).astype(BF16))
        for p, op in enumerate(ops):
            xn_ops[p] = pltpu.bitcast(op, U32)
        return ops

    def moments(z):
        z = z.reshape(CHUNK // SUBLANES, SUBLANES, LANES)
        mean = jnp.sum(z, axis=0) * (SUBLANES / CHUNK)
        return mean, jnp.sum((z - mean) * (z - mean), axis=0)

    def mix(j, first, n_rows, rhs, fetch):
        tail_a, tail_b = rhs[7][:, :D - 2 * KD], rhs[7][:, D - 2 * KD:]

        def keep_z2(i, c, z):
            z = _gelu(z)
            z2_v[i, c:c + CHUNK, :] = z
            moment_v[i, 0, c // CHUNK], moment_v[i, 1, c // CHUNK] = moments(z)
            start(itertools.islice(fetch, group * CHUNK * 3 // FH))

        for c in range(first, first + n_rows, CHUNK):
            lo, hi = slice(c, c + CHUNK), slice(FH + c, FH + c + CHUNK)
            m4 = _dot_nt(win_v[hi, KD:2 * KD], rhs[3])
            m2 = _dot_nt(win_ops[0, lo, :], rhs[1])
            keep_z2(j, c, _dot_nt(win_v[hi, 2 * KD:], tail_a) + (m2 + m4))
            m1 = _dot_nt(win_ops[2, lo, :], rhs[0])
            m3 = _dot_nt(win_v[lo, :KD], rhs[2])
            keep_z2(j + n_pairs, c,
                    _dot_nt(jnp.concatenate([win_ops[3, lo, :], win_v[hi, 2 * KD:]], axis=1),
                            jnp.concatenate([rhs[5], tail_b], axis=1)) + (m1 - m2 + m3))
            m5 = _dot_nt(win_ops[1, lo, :], rhs[4])
            z1_v[j + n_pairs, lo, :] = _dot_nt(win_v[lo, 2 * KD:], tail_b) + (m3 + m5)
            z1_v[j, lo, :] = (
                _dot_nt(jnp.concatenate([win_ops[4, lo, :], win_v[lo, 2 * KD:]], axis=1),
                        jnp.concatenate([rhs[6], tail_a], axis=1)) + (m1 + m4 - m5))

    def saved_operands():
        return [_as_bf16(xn_ops[p]) for p in range(8)]

    def prepare_win(c, n):
        ops = _left_operands(*(win_v[r + c:r + c + n, k * KD:(k + 1) * KD].astype(F32)
                               for r in (0, FH) for k in (0, 1)))
        for slot, p in enumerate((1, 4, 0, 5, 6)):
            win_ops[slot, c:c + n, :] = ops[p].astype(BF16)

    start(x_first + win_cp[0])
    wait(x_first)
    start(win_cp[1])
    rhs = mix_operands(0)
    for i, (c, n) in enumerate(win_spans):
        wait(win_cp[i])
        if i + 2 < len(win_spans):
            start(win_cp[i + 2])
        elif i + 2 == len(win_spans):
            start(x_rest)
        prepare_win(c, n)
        if c < half_f:
            mix(0, c, n, rhs, iter(()))
    wait(x_rest)
    start([wout_cp, b_cp, mem_cp] + wsp_copies(0) + wsp_copies(1))

    @pl.loop(1, n_pairs)
    def _(j):
        fetch = iter(wqkv_copies(j - 1))
        mix(j - 1, half_f, half_f, saved_operands(), fetch)
        mix(j, 0, half_f, mix_operands(j), fetch)
        start(fetch)

    fetch = iter(wqkv_copies(n_pairs - 1))
    mix(n_pairs - 1, half_f, half_f, saved_operands(), fetch)
    start(fetch)

    def merge_moments(i):
        means, m2s = moment_v[i, 0], moment_v[i, 1]
        groups = means.shape[0] * SUBLANES
        mean = jnp.sum(jnp.sum(means, axis=0), axis=0, keepdims=True) * (1.0 / groups)
        m2 = jnp.sum(m2s + (FH // groups) * ((means - mean) * (means - mean)), axis=0)
        return mean, lax.rsqrt(jnp.sum(m2, axis=0, keepdims=True) * (1.0 / FH) + LN_EPS)

    stats = [merge_moments(i) for i in range(n_blocks)]

    def new_spatial_operands(c):
        tiles = []
        for k in range(n_pairs):
            ops = _left_operands(*((z2_v[i, r:r + CHUNK, :] - stats[i][0]) * stats[i][1]
                                   for r in (c, half_f + c) for i in (k, k + n_pairs)))
            tiles.append([op.astype(BF16) for op in ops])
            for p in range(7):
                z2_ops[p, k, c // 2:(c + CHUNK) // 2, :] = pltpu.bitcast(tiles[k][p], U32)
        return [jnp.concatenate(op, axis=1) for op in zip(*tiles)]

    def saved_spatial_operands(c):
        return [jnp.concatenate([_as_bf16(z2_ops[p, k, c // 2:(c + CHUNK) // 2, :])
                                 for k in range(n_pairs)], axis=1) for p in range(7)]

    def prepare_wout():
        w = wout_v[...].astype(F32)
        lo, hi = w[:KF].T, w[KF:2 * KF].T
        ops = _left_operands(lo[:half_d], hi[:half_d], lo[half_d:], hi[half_d:])
        for p in range(7):
            wout_ops[p] = ops[p].astype(BF16)
        wout_rest[...] = w[2 * KF:].T.astype(BF16)

    def gate(j):
        rhs = _right_operands(gated_v[0, :KF, :], gated_v[1, :KF, :],
                              gated_v[0, KF:2 * KF, :], gated_v[1, KF:2 * KF, :])
        m = [_dot(wout_ops[p], rhs[p]) for p in range(7)]
        for i, top, bottom in ((0, m[0] + m[3] - m[4] + m[6], m[1] + m[3]),
                               (1, m[2] + m[4], m[0] - m[1] + m[2] + m[5])):
            y = _dot(wout_rest[...], gated_v[i, 2 * KF:, :]) + jnp.concatenate([top, bottom], axis=0)
            gate_v[rows(j + i * n_pairs), :] = _silu(y.T)

    def spatial(j, left_operands, previous_gate=None):
        wa, wb = wsp_v[rows(j), :].astype(F32), wsp_v[rows(j + n_pairs), :].astype(F32)
        rhs = _right_operands(wa[:, :S // 2], wb[:, :S // 2], wa[:, S // 2:], wb[:, S // 2:])
        rhs = [r.astype(BF16) for r in rhs]
        for c in range(0, half_f, CHUNK):
            lhs = left_operands(c)
            m = [None] * 7
            for p in (3, 1, 2, 4, 0, 5, 6):
                m[p] = _dot_nt(lhs[p], rhs[p])
            if c == 0 and previous_gate:
                previous_gate()
            for i, r, g in ((0, half_f + c, m[1] + m[3]),
                            (1, c, m[2] + m[4]),
                            (1, half_f + c, m[0] - m[1] + m[2] + m[5]),
                            (0, c, m[0] + m[3] - m[4] + m[6])):
                block = j + i * n_pairs
                gated_v[i, r:r + CHUNK, :] = (_gelu(z1_v[block, r:r + CHUNK, :])
                                              * (g + bias_v[pl.ds(block, 1), :]))

    wait([wout_cp, b_cp] + wsp_copies(0))
    start(wsp_copies(2))
    bias_v[...] = b_v[...].astype(F32)
    prepare_wout()
    spatial(0, new_spatial_operands)

    @pl.loop(1, n_pairs)
    def _(j):
        @pl.when(j + 2 < n_pairs)
        def _():
            start(wsp_copies(j + 2) + [wo_copy(j - 1)])

        wait(wsp_copies(j))
        spatial(j, saved_spatial_operands, functools.partial(gate, j - 1))

    start([wo_copy(n) for n in range(n_pairs - 3, d_tiles)])
    wait([mem_cp] + [wo_copy(n) for n in range(d_tiles)])
    pltpu.make_async_copy(wqkv_v, wqkv_v, wqkv_sem.at[0]).wait()
    gate(n_pairs - 1)

    wo_w = wo_v.bitcast(U32)

    scale = LANES ** -0.5
    early = H // 2
    k_head = (d_tiles - 1) * LANES

    def saved_weights(i):
        return [wqkv_v.at[m, i] for m in range(3)]

    def repacked_weights():
        heads = []
        for i in range(0, H, 2):
            even, odd = ([wqkv_v[m, i + par] for m in range(3)] for par in range(2))
            heads.append([(a & 0xFFFF) | (b << 16) for a, b in zip(even, odd)])
            heads.append([(a >> 16) | (b & jnp.uint32(0xFFFF0000)) for a, b in zip(even, odd)])
            for m in range(3):
                wqkv_v[m, i], wqkv_v[m, i + 1] = heads[i][m], heads[i + 1][m]
            yield heads[i]
            yield heads[i + 1]

    def step(r0, mem, weights):
        row_id = lax.broadcasted_iota(jnp.int32, (L, L), 0)
        col_id = lax.broadcasted_iota(jnp.int32, (L, L), 1)
        visible = (row_id < M) | (row_id >= col_id)
        h = jnp.concatenate([mem, xn_v[pl.ds(r0, seg), :]], axis=0)
        q, k, v, e, inv, o = ([None] * H for _ in range(6))
        first = next(weights)
        part = [_dot(h[:, :k_head], _as_bf16(w[:k_head // 2, :])) for w in first]
        q[0], k[0], v[0] = (
            _dot(h[:, k_head:], _as_bf16(w[k_head // 2:, :])) + p for w, p in zip(first, part))
        head_sum = []
        for i in range(H + PV_DELAY):
            if 0 < i < H:
                q[i], k[i], v[i] = (_dot(h, _as_bf16(w[...])) for w in next(weights))
            if i >= H:
                o_early = jnp.concatenate(o[:early], axis=1)
                while len(head_sum) < (i - H + 1) * d_tiles // PV_DELAY:
                    n = len(head_sum)
                    head_sum.append(_dot(o_early, _as_bf16(wo_w[n, :early * LANES // 2, :])))
            j = i - QK_DELAY
            if 0 <= j < H:
                sc = jnp.where(visible, _dot_nt(q[j], k[j]) * scale, MASK_VALUE)
                e[j] = jnp.exp(sc - jnp.max(sc, axis=-1, keepdims=True))
                denom = jnp.sum(e[j], axis=-1, keepdims=True)
                r = pltpu.reciprocal(denom, approx=True)
                inv[j] = r * (2.0 - denom * r)
            j = i - PV_DELAY
            if 0 <= j < H:
                o[j] = _dot(e[j], v[j]) * inv[j]
        o_late = jnp.concatenate(o[early:], axis=1)
        y = jnp.concatenate(
            [_dot(o_late, _as_bf16(wo_w[n, early * LANES // 2:, :])) + head_sum[n]
             for n in range(d_tiles)], axis=1)
        res = x_v[pl.ds(r0, seg), :].astype(F32) + y[M:, :] * gate_v[pl.ds(r0, seg), :]
        out_v[pl.ds(r0, seg), :] = res.astype(BF16)
        return y[:M, :]

    chunk = STEP_UNROLL * seg

    def out_copy(start, n):
        return pltpu.make_async_copy(out_v.at[pl.ds(start, n)], out_hbm.at[pl.ds(start, n)],
                                     out_sem.at[0])

    def body(it, mem):
        @pl.when(it > 0)
        def _():
            out_copy(pl.multiple_of((it - 1) * chunk, chunk), chunk).start()

        base = pl.multiple_of(seg + it * chunk, seg)
        for u in range(STEP_UNROLL):
            mem = step(pl.multiple_of(base + u * seg, seg), mem, map(saved_weights, range(H)))
        return mem

    mem = step(0, mem_v[...].astype(F32), repacked_weights())
    n_trips = (n_seg - 1) // STEP_UNROLL
    if not SKIP3:
        lax.fori_loop(0, n_trips, body, mem)
        sent = (n_trips - 1) * chunk
    else:
        sent = 0
    out_copy(sent, S - sent).start()
    out_copy(0, S).wait()


@functools.partial(jax.jit, static_argnames=("A_seg_len",))
def pallas_recurrent_scan__memory_aug_recurrent_mem_tr__mixer_gmlp__prompt_kernel(
    A_x: jax.Array,
    A_mem0: jax.Array,
    A_Wq: jax.Array,
    A_Wk: jax.Array,
    A_Wv: jax.Array,
    A_Wo: jax.Array,
    A_seg_len: int,
    B_x: jax.Array,
    B_w_in: jax.Array,
    B_w_sp: jax.Array,
    B_b_sp: jax.Array,
    B_w_out: jax.Array,
):
    del B_x
    B, S, D = A_x.shape
    M = A_mem0.shape[1]
    _, H, Dh = A_Wq.shape
    F = B_w_in.shape[1]
    FH = F // 2
    seg = int(A_seg_len)
    assert B == 1 and Dh == LANES and D % LANES == 0 and H % 2 == 0
    assert S % (2 * LANES) == 0 and (S // seg - 1) % STEP_UNROLL == 0
    KD = D // (2 * LANES) * LANES
    KF = FH // (2 * LANES) * LANES

    hbm = pl.BlockSpec(memory_space=pltpu.HBM)
    out = pl.pallas_call(
        functools.partial(_kernel, seg=seg),
        out_shape=jax.ShapeDtypeStruct((S, D), BF16),
        in_specs=[hbm] * 10,
        out_specs=hbm,
        scratch_shapes=[
            pltpu.VMEM((S, D), BF16),
            pltpu.VMEM((M, D), BF16),
            pltpu.VMEM((3, H, D // 2, LANES), U32),
            pltpu.VMEM((D // LANES, H * Dh, LANES), BF16),
            pltpu.VMEM((F, D), BF16),
            pltpu.VMEM((S, S), BF16),
            pltpu.VMEM((S // LANES, LANES), BF16),
            pltpu.VMEM((FH, D), BF16),
            pltpu.VMEM((S, D), F32),
            pltpu.VMEM((8, LANES // 2, KD), U32),
            pltpu.VMEM((5, FH, KD), BF16),
            pltpu.VMEM((S // LANES, FH, LANES), F32),
            pltpu.VMEM((S // LANES, FH, LANES), F32),
            pltpu.VMEM((S // LANES, 2, FH // CHUNK, SUBLANES, LANES), F32),
            pltpu.VMEM((S // LANES, LANES), F32),
            pltpu.VMEM((7, S // (2 * LANES), FH // 4, LANES), U32),
            pltpu.VMEM((2, FH, LANES), F32),
            pltpu.VMEM((7, D // 2, KF), BF16),
            pltpu.VMEM((D, FH - 2 * KF), BF16),
            pltpu.VMEM((S, D), F32),
            pltpu.VMEM((S, D), BF16),
            pltpu.SemaphoreType.DMA((2,)),
            pltpu.SemaphoreType.DMA((FH // 2 // CHUNK + 1,)),
            pltpu.SemaphoreType.DMA((S // (2 * LANES),)),
            pltpu.SemaphoreType.DMA((1,)),
            pltpu.SemaphoreType.DMA((5,)),
            pltpu.SemaphoreType.DMA((1,)),
        ],
        compiler_params=pltpu.CompilerParams(
            vmem_limit_bytes=110 * 1024 * 1024, flags=FLAGS),
    )(
        A_x.reshape(S, D),
        A_mem0.reshape(M, D),
        A_Wq.reshape(D // 2, 2, H, Dh),
        A_Wk.reshape(D // 2, 2, H, Dh),
        A_Wv.reshape(D // 2, 2, H, Dh),
        A_Wo.reshape(H * Dh, D),
        B_w_in.T,
        B_w_sp,
        B_b_sp.reshape(S // LANES, LANES),
        B_w_out,
    )
    return out.reshape(B, S, D)
```

```python
import functools
import itertools

import jax
import jax.numpy as jnp
from jax import lax
import jax.experimental.pallas as pl
import jax.experimental.pallas.tpu as pltpu

F32 = jnp.float32
BF16 = jnp.bfloat16
U32 = jnp.uint32

LANES = 128
SUBLANES = 8
SLAB = 16
CHUNK = 144
STEP_UNROLL = 4
GATE_PIECES = 91
VALUE_DELAY = 3
LN_EPS = 1e-5
MASK_VALUE = -1000000000.0
VMEM_LIMIT = 126 * 1024 * 1024


def _dot(a, b):
    return jnp.dot(a, b, preferred_element_type=F32)


def _dot_nt(a, b):
    return lax.dot_general(a, b, (((1,), (1,)), ((), ())), preferred_element_type=F32)


def _as_bf16(words):
    return pltpu.bitcast(words, BF16)


def _layernorm(v):
    n = v.shape[-1]
    mean = jnp.sum(v, axis=-1, keepdims=True) * (1.0 / n)
    c = v - mean
    var = jnp.sum(c * c, axis=-1, keepdims=True) * (1.0 / n)
    return c * lax.rsqrt(var + LN_EPS)


def _gelu(v):
    inner = v * (0.7978845608028654 + (0.7978845608028654 * 0.044715) * (v * v))
    half = 0.5 * v
    return half + half * jnp.tanh(inner)


def _silu(v):
    half = 0.5 * v
    return half + half * jnp.tanh(half)


def _left_operands(a11, a12, a21, a22):
    return (a11 + a22, a21 + a22, a11, a22, a11 + a12, a21 - a11, a12 - a22)


def _right_operands(b11, b12, b21, b22):
    return (b11 + b22, b11, b12 - b22, b21 - b11, b22, b11 + b12, b21 + b22)


_BLOCK_TERMS = (((0, 1), (3, 1), (4, -1), (6, 1)),
                ((2, 1), (4, 1)),
                ((1, 1), (3, 1)),
                ((0, 1), (2, 1), (5, 1), (1, -1)))
_PRODUCT_ORDER = (3, 1, 2, 4, 0, 5, 6)


def _result_block(c, products):
    return _signed_sum([(sign, products[p]) for p, sign in _BLOCK_TERMS[c]])


_TILES = 5
_PRODUCTS = tuple(
    tuple(tuple((int(term[-2]), int(term[-1]), -1 if term[0] == "-" else 1)
                for term in terms.replace("-", "+-").split("+") if term)
          for terms in entry.split())
    for entry in (
        "00-10 03-02+42-30+00-04-10 00",
        "01 11-01-12-14-31 01",
        "02 03-02+42+22-21-24-32 02+12",
        "03-13 33-13-32-34 03",
        "04 44-04-34-41 04+14",
        "00+01 01 00+01+10+11",
        "00+02 02-03-42 00+02",
        "00+04 04-42 00+04",
        "01+02-11-12 12 01+02",
        "01+03 31 01+03+11+13",
        "01+04-11-14 14 01+04",
        "02+03 32-03 02+03",
        "03+04 34 03+04",
        "00+02+03 03 00+02+03+10+12+13",
        "00+02+04-10-12-14 42 00+02+04",
        "10 00+24+30-01-03-20-40 00+10",
        "11 11-10-13-21-41 11",
        "02-12 20-24-30+12+23+42-22 12",
        "13 33-23-31-43 03+13",
        "04-14 14+40+43-44 14",
        "00+01-10-11 10 -10-11",
        "10+12 20-24-30 10+12",
        "10+14 40-24 10+14",
        "11+12 21 01+02+11+12",
        "01+03-11-13 13 -11-13",
        "11+14 41 01+04+11+14",
        "12+13 23-30 12+13",
        "13+14 43 13+14",
        "00+02+03-10-12-13 30 -10-12-13",
        "10+12+14 24 00+02+04+10+12+14",
        "00+01-10 10-01 00+10+11",
        "02+10 03-02+42-30+20-24 00-12",
        "04+10 40-04 00-14",
        "02-11-12 12-21 -01-02-12",
        "01+03-13 13-31 03+11+13",
        "04-11-14 14-41 -01-04-14",
        "02+13 32-23 -03+12",
        "04+13 43-34 03-14",
        "00+02+03-10 30-03 00+10+12+13",
        "02-10-12-14 24-42 00+02+04+12",
        "00 01-11 01+11", "00+01 11 01-00", "01-11 10+11 00", "02 21-31 01+11",
        "02+03 31 01-00", "03-13 30+31 00", "04 40 00", "04 41 01",
        "10+11 00 10-11", "11 10-00 00+10", "10-00 00+01 11", "12+13 20 10-11",
        "13 30-20 00+10", "12-02 20+21 11", "14 40 10", "14 41 11",
        "00+11 00+11 00+11", "02+13 20+31 00+11",
        "00 01-11 01+11", "00+01 11 01-00", "01-11 10+11 00", "00 03-13 03+13",
        "00+01 13 03-02", "01-11 12+13 02", "00 04 04", "01 14 04",
        "10+11 00 10-11", "11 10-00 00+10", "10-00 00+01 11", "10+11 02 12-13",
        "11 12-02 02+12", "10-00 02+03 13", "10 04 14", "11 14 14",
        "00+11 00+11 00+11", "00+11 02+13 02+13",
    ))
_GROUP = (range(0, 15), range(15, 30), range(30, 40))
_PAIR_IN = (range(40, 48), range(48, 56), range(56, 58))
_PAIR_OUT = (range(58, 66), range(66, 74), range(74, 76))
_PARTS = ((0, 2, 6, 15, 17, 21, 22, 29, 31, 39), (4, 7, 10, 12, 14, 19, 25, 32, 35, 37),
          (1, 5, 8, 9, 16, 20, 23, 30, 33, 34), (3, 11, 13, 18, 24, 26, 27, 28, 36, 38))


def _signed_sum(terms, total=None):
    if total is None:
        first = max(range(len(terms)), key=lambda i: terms[i][0])
        terms = [terms[first]] + terms[:first] + terms[first + 1:]
    for sign, v in terms:
        if total is None:
            total = v if sign > 0 else -v
        else:
            total = total + v if sign > 0 else total - v
    return total


def _slot(g, p):
    first = max(top[0] for top, _, _ in (_GROUP, _PAIR_IN, _PAIR_OUT) if top[0] <= p)
    return g * _GROUP[2].stop + p - first


def _factor(p, side, block):
    return _signed_sum([(sign, block(i, j)) for i, j, sign in _PRODUCTS[p][side]
                        if block(i, j) is not None])


def _collect(i, j, products, total=None):
    return _signed_sum([(sign, v) for p, v in products.items()
                        for r, c, sign in _PRODUCTS[p][2] if (r, c) == (i, j)], total)


def _blocks_fed_by(products):
    return sorted({(i, j) for p in products for i, j, _ in _PRODUCTS[p][2]})


def _after(result, never, value):
    return jnp.where(never, pltpu.bitcast(result, U32), jnp.uint32(value))


def _pacer(pieces, n_matmuls):
    side_work, share = iter(pieces), pl.cdiv(len(pieces), n_matmuls) or 1

    def trail(result):
        step = max(1, result.shape[0] // SUBLANES // share)
        for i, piece in zip(range(share), side_work):
            row = min(i * step * SUBLANES, result.shape[0] - SUBLANES)
            piece(result[row:row + SUBLANES, :LANES])
        return result

    return trail


def _kernel(
    x_hbm, mem_hbm, wq_hbm, wk_hbm, wv_hbm, wo_hbm, win_hbm, wsp_hbm, b_hbm, wout_hbm,
    out_hbm,
    x_v, words_v, wqkv_ops, wo_ops, wo_v, xn_v, gate_v, qkv_part, mem_v,
    x_sem, win_sem, wsp_sem, weight_sem, misc_sem, out_sem,
    *, seg,
):
    S, D = x_v.shape
    M = mem_hbm.shape[0]
    H = 2 * words_v.shape[1]
    FH = wout_hbm.shape[0]
    n_blocks = S // LANES
    G = H // _TILES
    n_pairs = n_blocks // 2
    n_quads = n_blocks // 4
    n_seg = S // seg
    d_tiles = D // LANES
    L = M + seg

    KD = d_tiles // 2 * LANES
    KF = FH // (2 * LANES) * LANES
    half_f = FH // 2
    half_d = D // 2
    batch = 2 * _TILES

    def rows(i):
        start = i * LANES
        return pl.ds(start if isinstance(i, int) else pl.multiple_of(start, LANES), LANES)

    def x_copies(j):
        return [pltpu.make_async_copy(x_hbm.at[rows(i)], x_v.at[rows(i)], x_sem.at[j])
                for i in (j, j + n_pairs)]

    def qkv_copies(i, sem):
        return [pltpu.make_async_copy(w_hbm.bitcast(U32).at[:, i, :], words_v.at[m, i],
                                      weight_sem.at[sem])
                for m, w_hbm in enumerate((wq_hbm, wk_hbm, wv_hbm))]

    def wait_for_qkv(j, n_heads):
        words = words_v.at[:, pl.ds(j * (batch // 2), n_heads // 2)]
        pltpu.make_async_copy(words, words, weight_sem.at[j]).wait()

    mem_cp = pltpu.make_async_copy(mem_hbm, mem_v.at[0], misc_sem.at[3])
    wo_cp = [pltpu.make_async_copy(wo_hbm.at[:, rows(n)], wo_v.at[n], misc_sem.at[4])
             for n in range(d_tiles)]

    def start(copies):
        for cp in copies:
            cp.start()

    def wait(copies):
        for cp in copies:
            cp.wait()

    def cols(k, n=1):
        return slice(k * LANES, (k + n) * LANES)

    def tokens(t):
        return lambda i, k: t[i * seg // 2:(i + 1) * seg // 2, cols(k)]

    def prepare_qkv(j, m, u, r, part, never, result):
        unpack = [jnp.concatenate([_after(result, never, v)] * (SLAB // SUBLANES), axis=0)
                  for v in (16, 0xFFFF0000)]

        def tile(k, n):
            h = _TILES * u + n
            words = words_v[m, j * _TILES + h // 2, pl.ds(k * LANES + r, SLAB), :]
            return pltpu.bitcast(words & unpack[1] if h % 2 else words << unpack[0], F32)

        tiles = {(k, n): tile(k, n) for p in part for k, n, _ in _PRODUCTS[p][1]}
        for p in part:
            op = _factor(p, 1, lambda k, n: tiles[k, n])
            wqkv_ops[m, _slot(2 * j + u, p), r:r + SLAB, :] = op.astype(BF16)

    def prepare_wo(g, r, part, never, result):
        zero = _after(result, never, 0)

        def tile(k, n):
            first = ((_TILES * g + k) * LANES + r) // 2
            words = wo_v.bitcast(U32)[n, first:first + SLAB // 2, :]
            return _as_bf16(words | zero).astype(F32)

        tiles = {(k, n): tile(k, n) for p in part for k, n, _ in _PRODUCTS[p][1]}
        for p in part:
            op = _factor(p, 1, lambda k, n: tiles[k, n])
            wo_ops[_slot(g, p), r:r + SLAB, :] = op.astype(BF16)

    def gmlp(win_v, wsp_v, xn_ops, win_ops, z1_v, z2_v, z2_ops, gated_v, wout_ops, wout_rest,
             wout_v, moment_v, stat_v, b_v, bias_v):
        def wsp_copies(j):
            return [pltpu.make_async_copy(wsp_hbm.at[rows(j + i)], wsp_v.at[rows(j + i)],
                                          wsp_sem.at[j]) for i in range(0, n_blocks, n_quads)]

        win_cp = [[pltpu.make_async_copy(win_hbm.at[pl.ds(r + c, CHUNK)], win_v.at[pl.ds(r + c, CHUNK)],
                                         win_sem.at[c // CHUNK]) for r in (FH, 0)]
                  for c in range(0, FH, CHUNK)]
        b_cp = pltpu.make_async_copy(b_hbm, b_v, misc_sem.at[1])
        wout_cp = pltpu.make_async_copy(wout_hbm, wout_v, misc_sem.at[2])

        def mix_operands(j):
            xa, xb = (_layernorm(x_v[rows(i), :].astype(F32)) for i in (j, j + n_pairs))
            xn_v[rows(j), :] = xa
            xn_v[rows(j + n_pairs), :] = xb
            ops = _right_operands(xa[:, :KD], xb[:, :KD], xa[:, KD:2 * KD], xb[:, KD:2 * KD])
            ops = [op.astype(BF16) for op in ops]
            ops.append(jnp.concatenate([xa[:, 2 * KD:], xb[:, 2 * KD:]], axis=1).astype(BF16))
            for p, op in enumerate(ops):
                xn_ops[p] = pltpu.bitcast(op, U32)
            return ops

        def moments(z):
            z = z.reshape(CHUNK // SUBLANES, SUBLANES, LANES)
            mean = jnp.sum(z, axis=0) * (SUBLANES / CHUNK)
            return mean, jnp.sum((z - mean) * (z - mean), axis=0)

        def mix(j, first, n_rows, rhs, fetch=()):
            tail_a, tail_b = rhs[7][:, :D - 2 * KD], rhs[7][:, D - 2 * KD:]

            found = []

            def keep_z2(i, c, z):
                z = _gelu(z)
                z2_v[i, c:c + CHUNK, :] = z
                found.append(moments(z))
                start(itertools.islice(fetch, 1))

            for c in range(first, first + n_rows, CHUNK):
                lo, hi = slice(c, c + CHUNK), slice(FH + c, FH + c + CHUNK)
                m4 = _dot_nt(win_v[hi, KD:2 * KD], rhs[3])
                m2 = _dot_nt(win_ops[0, lo, :], rhs[1])
                keep_z2(j, c, _dot_nt(win_v[hi, 2 * KD:], tail_a) + (m2 + m4))
                m1 = _dot_nt(win_ops[2, lo, :], rhs[0])
                m3 = _dot_nt(win_v[lo, :KD], rhs[2])
                keep_z2(j + n_pairs, c,
                        _dot_nt(jnp.concatenate([win_ops[3, lo, :], win_v[hi, 2 * KD:]], axis=1),
                                jnp.concatenate([rhs[5], tail_b], axis=1)) + (m1 - m2 + m3))
                m5 = _dot_nt(win_ops[1, lo, :], rhs[4])
                z1_v[j + n_pairs, lo, :] = _dot_nt(win_v[lo, 2 * KD:], tail_b) + (m3 + m5)
                z1_v[j, lo, :] = (
                    _dot_nt(jnp.concatenate([win_ops[4, lo, :], win_v[lo, 2 * KD:]], axis=1),
                            jnp.concatenate([rhs[6], tail_a], axis=1)) + (m1 + m4 - m5))
            return found

        def save_moments(found):
            for n, (mean, m2) in enumerate(found):
                moment_v[n, 0], moment_v[n, 1] = mean, m2

        def merge_moments(j, found):
            for i, parts in ((j, found[0::2]), (j + n_pairs, found[1::2])):
                means, m2s = zip(*parts)
                groups = len(parts) * SUBLANES
                mean = jnp.sum(sum(means), axis=0, keepdims=True) * (1.0 / groups)
                spread = sum((m - mean) * (m - mean) for m in means)
                m2 = jnp.sum(sum(m2s) + (FH // groups) * spread, axis=0, keepdims=True)
                stat_v[i, 0:1, :] = mean
                stat_v[i, 1:2, :] = lax.rsqrt(m2 * (1.0 / FH) + LN_EPS)

        def finish(j, fetch):
            found = [(moment_v[n, 0], moment_v[n, 1]) for n in range(moment_v.shape[0])]
            merge_moments(j, found + mix(j, half_f, half_f, saved_operands(), fetch))

        def saved_operands():
            return [_as_bf16(xn_ops[p]) for p in range(8)]

        def prepare_wout(t):
            lo, hi = (wout_v[rows(i), :].astype(F32).T for i in (t, t + KF // LANES))
            ops = _left_operands(lo[:half_d], hi[:half_d], lo[half_d:], hi[half_d:])
            for p in range(7):
                wout_ops[p, t] = pltpu.bitcast(ops[p].astype(BF16), U32)

        def advance(j):
            fetch = iter(qkv_copies(j - 2, lax.div(j - 2, batch // 2)))
            finish(j - 1, fetch)
            save_moments(mix(j, 0, half_f, mix_operands(j), fetch))
            start(fetch)

        queue = win_cp[2:] + [x_copies(1), x_copies(2) + x_copies(3) + [wout_cp],
                              [cp for j in range(4, n_pairs) for cp in x_copies(j)]]
        start(x_copies(0) + win_cp[0])
        wait(x_copies(0))
        start(win_cp[1] + queue.pop(0))
        rhs = mix_operands(0)
        found = []
        for c in range(0, FH, CHUNK):
            wait(win_cp[c // CHUNK])
            start(queue.pop(0))
            ops = _left_operands(*(win_v[r + c:r + c + CHUNK, k * KD:(k + 1) * KD].astype(F32)
                                   for r in (0, FH) for k in (0, 1)))
            for slot, p in enumerate((1, 4, 0, 5, 6)):
                win_ops[slot, c:c + CHUNK, :] = ops[p].astype(BF16)
            found += mix(0, c, CHUNK, rhs)
            if c == FH - 2 * CHUNK:
                wait(x_copies(1))
        merge_moments(0, found)
        save_moments(mix(1, 0, half_f, mix_operands(1)))
        start([b_cp] + wsp_copies(0))
        wout_cp.wait()

        @pl.loop(2, n_pairs, step=2)
        def _(j):
            wait(x_copies(j) + x_copies(j + 1))
            advance(j)
            advance(j + 1)
            prepare_wout(j // 2 - 1)

        def new_spatial_operands():
            tiles = []
            for k in range(n_pairs):
                tiles.append(_left_operands(*(
                    (z2_v[i, r:r + half_f, :] - stat_v[i, 0:1, :]) * stat_v[i, 1:2, :]
                    for r in (0, half_f) for i in (k, k + n_pairs))))
                for p in range(7):
                    z2_ops[p, k] = tiles[k][p]
            return lambda p, k, r: tiles[k][p][r:r + half_f // 2]

        def saved_spatial_operands(p, k, r):
            return z2_ops[p, k, r:r + half_f // 2, :]

        def gate(j, u, pieces):
            rhs = _right_operands(gated_v[u, 0, :KF, :], gated_v[u, 1, :KF, :],
                                  gated_v[u, 0, KF:2 * KF, :], gated_v[u, 1, KF:2 * KF, :])
            trail = _pacer(pieces, 7)
            m = {p: trail(_dot(jnp.concatenate(
                [_as_bf16(wout_ops[p, t]) for t in range(KF // LANES)], axis=1), rhs[p]))
                for p in range(7)}
            c11, c12, c21, c22 = (_result_block(c, m) for c in range(4))
            for i, top, bottom in ((0, c11, c21), (1, c12, c22)):
                y = (_dot(wout_rest[...], gated_v[u, i, 2 * KF:, :])
                     + jnp.concatenate([top, bottom], axis=0))
                gate_v[rows(j + i * n_pairs), :] = _silu(y.T)

        def spatial(j, left, pieces=()):
            rhs = []
            for pair in (j, j + n_quads):
                wa, wb = (wsp_v[rows(i), :].astype(F32) for i in (pair, pair + n_pairs))
                rhs.append(_right_operands(wa[:, :S // 2], wb[:, :S // 2],
                                           wa[:, S // 2:], wb[:, S // 2:]))

            trail = _pacer(pieces, 7 * 7)

            def product(p):
                lhs = _left_operands(*(
                    jnp.concatenate([left(p, k0 + k, r) for k in range(n_quads)], axis=1)
                    for r in (0, half_f // 2) for k0 in (0, n_quads)))
                wa, wb = rhs[0][p], rhs[1][p]
                ops = _right_operands(wa[:, :S // 4], wb[:, :S // 4],
                                      wa[:, S // 4:], wb[:, S // 4:])
                n = {i: trail(_dot_nt(lhs[i], ops[i])) for i in _PRODUCT_ORDER}
                c11, c12, c21, c22 = (_result_block(c, n) for c in range(4))
                return {(0, half_f // 2): c21, (1, 0): c12, (1, half_f // 2): c22, (0, 0): c11}

            m = {}
            ready_after = {1: 2, 4: 1, 5: 3, 6: 0}
            for p in _PRODUCT_ORDER:
                m[p] = product(p)
                if p in ready_after:
                    row_half, i = divmod(ready_after[p], 2)
                    for u, r in m[p]:
                        g = _result_block(ready_after[p], {q: m[q][u, r] for q in m})
                        block = j + u * n_quads + i * n_pairs
                        span = slice(row_half * half_f + r, row_half * half_f + r + half_f // 2)
                        gated_v[u, i, span, :] = (_gelu(z1_v[block, span, :])
                                                  * (g + bias_v[pl.ds(block, 1), :]))

        wait([b_cp] + wsp_copies(0))
        start(wsp_copies(1))
        bias_v[...] = b_v[...].astype(F32)
        fetch = iter([cp for i in range(n_pairs - 2, batch)
                      for cp in qkv_copies(i, i // (batch // 2))])
        wout_rest[...] = wout_v[2 * KF:, :].astype(F32).T.astype(BF16)
        finish(n_pairs - 1, fetch)
        start(fetch)
        spatial(0, new_spatial_operands())

        @pl.loop(1, n_quads)
        def _(j):
            @pl.when(j + 1 < n_quads)
            def _():
                start(wsp_copies(j + 1))
                share = (H // 2 - batch) // (n_quads - 2)
                for i in range(share):
                    pair = batch + (j - 1) * share + i
                    start(qkv_copies(pair, lax.div(pair, batch // 2)))

            @pl.when(j + 1 == n_quads)
            def _():
                start(wo_cp + [mem_cp])

            wait(wsp_copies(j))
            wait_for_qkv(j - 1, batch)
            never = jnp.full((SUBLANES, LANES), j) < 0
            pieces = [functools.partial(prepare_qkv, j - 1, m, u, r, part, never) for m in range(3)
                      for u in range(2) for r in range(0, LANES, SLAB) for part in _PARTS]
            gate(j - 1, 0, pieces[:GATE_PIECES])
            gate(j - 1 + n_quads, 1, pieces[GATE_PIECES:2 * GATE_PIECES])
            spatial(j, saved_spatial_operands, pieces[2 * GATE_PIECES:])

        wait(wo_cp)
        wait_for_qkv(n_quads - 1, H - (n_quads - 1) * batch)
        never = jnp.exp(bias_v[:SUBLANES, :]) < 0
        pair_in, pair_out = (tuple(itertools.chain(*some)) for some in (_PAIR_IN, _PAIR_OUT))
        pieces = []
        for r in range(0, LANES, SLAB):
            pieces += [functools.partial(prepare_qkv, G // 2, m, 0, r, pair_in, never)
                       for m in range(3)]
            pieces.append(functools.partial(prepare_wo, G, r, pair_out, never))
        pieces += [functools.partial(prepare_wo, g, r, part, never)
                   for g in range(G) for r in range(0, LANES, SLAB) for part in _PARTS]

        def first_visit(g, pieces):
            products = (_GROUP if g < G else _PAIR_IN)[1]
            trail = _pacer(pieces, 3 * len(products))
            for m in range(3):
                done = {p: trail(_dot(_factor(p, 0, tokens(xn_v[:seg, :])),
                                      _as_bf16(wqkv_ops.bitcast(U32)[m, _slot(g, p)])))
                        for p in products}
                for i, c in enumerate(_blocks_fed_by(done)):
                    qkv_part[0, m, g, i] = _collect(*c, done)

        gate(n_quads - 1, 0, pieces[:GATE_PIECES])
        for g in range(G + 1):
            if g == G // 2:
                gate(n_pairs - 1, 1, pieces[GATE_PIECES:2 * GATE_PIECES])
            first_visit(g, pieces[2 * GATE_PIECES + g::G + 1])

    def recurrence(out_v, o_v, y_part):
        half = seg // 2
        scale = LANES ** -0.5
        wqkv_w, wo_w = wqkv_ops.bitcast(U32), wo_ops.bitcast(U32)

        def finish_output(r0, parity, late):
            y = jnp.concatenate([
                jnp.concatenate([_collect(i, n, late, y_part[parity, i, n]) for n in range(_TILES)],
                                axis=1) for i in range(2)], axis=0)
            span = pl.ds(pl.multiple_of(r0, seg), seg)
            out_v[span, :] = (x_v[span, :].astype(F32) + y * gate_v[span, :]).astype(BF16)

        def step(r0, parity, mem):
            def in_order(products):
                long, short = list(products[parity]), list(products[2])
                if products is _GROUP:
                    def last_column(p):
                        return max(k for i, k, _ in _PRODUCTS[p][0] if i == parity)

                    pools = [iter(sorted(some, key=last_column)) for some in (long, short)]
                    return [next(pools[i]) for i in (0, 0, 1, 0, 1) * _TILES]
                return long[:2] + short[:1] + long[2:5] + short[1:] + long[5:]

            row_id = lax.broadcasted_iota(jnp.int32, (L, L), 0)
            col_id = lax.broadcasted_iota(jnp.int32, (L, L), 1)
            visible = (row_id < M) | (row_id >= col_id)

            def memory(t):
                return lambda i, k: t[:, cols(k)] if i == parity else None

            xs = xn_v[pl.ds(pl.multiple_of(r0, seg), seg), :]
            xs_next = xn_v[pl.ds(pl.multiple_of(jnp.minimum(r0 + seg, S - seg), seg), seg), :]
            lhs = {p: jnp.concatenate(
                [_factor(p, 0, tokens(xs))]
                + ([_factor(p, 0, tokens(xs_next))] if p in products[parity] else [])
                + [_factor(p, 0, memory(mem))], axis=0)
                for products in (_GROUP, _PAIR_IN) for p in in_order(products)}
            qkv, e, inv, o, sums = {}, {}, {}, {}, {}
            heads = [*range(_TILES * G, H), *range(_TILES * G)]

            def project(m, g):
                products = _GROUP if g < G else _PAIR_IN
                own = products[parity]
                done = {p: _dot(lhs[p], _as_bf16(wqkv_w[m, _slot(g, p)]))
                        for p in in_order(products)}
                earlier = {c: qkv_part[parity, m, g, i]
                           for i, c in enumerate(_blocks_fed_by(products[1 - parity]))}
                for i, c in enumerate(_blocks_fed_by(own)):
                    qkv_part[1 - parity, m, g, i] = _collect(
                        *c, {p: done[p][half:seg] for p in own})
                for n in range(min(_TILES, H - _TILES * g)):
                    qkv[m, _TILES * g + n] = jnp.concatenate(
                        [_collect(parity, n, {p: v[-M:] for p, v in done.items()})]
                        + [_collect(i, n, {p: v[:half] for p, v in done.items()},
                                    earlier.get((i, n))) for i in range(2)], axis=0)

            def attend(n_heads):
                for h in heads[len(e):n_heads]:
                    sc = jnp.where(visible, _dot_nt(qkv[0, h], qkv[1, h]) * scale, MASK_VALUE)
                    e[h] = jnp.exp(sc - jnp.max(sc, axis=-1, keepdims=True))
                    denom = jnp.sum(e[h], axis=-1, keepdims=True)
                    r = pltpu.reciprocal(denom, approx=True)
                    inv[h] = r * (2.0 - denom * r)

            def gather(n_heads):
                for h in heads[len(o):n_heads]:
                    o[h] = _dot(e[h], qkv[2, h]) * inv[h]
                    o_v[parity, :, cols(h)] = o[h][M:]

            def output_pass(g):
                products = _GROUP if g < G else _PAIR_OUT
                members = range(_TILES * g, min(H, _TILES * (g + 1)))
                now = jnp.concatenate([o[h] for h in members], axis=1)
                before = o_v[1 - parity, :, cols(members[0], len(members))]
                for p in in_order(products):
                    left = [_factor(p, 0, memory(now[:M])), _factor(p, 0, tokens(now[M:]))]
                    if p in products[parity]:
                        left.append(_factor(p, 0, tokens(before)))
                    d = _dot(jnp.concatenate(left, axis=0), _as_bf16(wo_w[_slot(g, p)]))
                    sums[p] = d + sums[p] if p in sums else d

            def n_ready(turn):
                if turn < 2:
                    return max(0, turn + 1)
                return H - _TILES * G + pl.cdiv(_TILES * (turn - 1), 3)

            for m in range(3):
                project(m, G)
            for turn in range(3 * G):
                project(turn % 3, turn // 3)
                attend(n_ready(turn))
                gather(n_ready(turn - VALUE_DELAY))
            for g in range(G + 1):
                output_pass(g)
                if g == 0:
                    attend(H)
                elif g == G - 4:
                    gather(n_ready(3 * G - 1))
                elif g == G - 3:
                    gather(H)

            finish_output(jnp.maximum(r0 - seg, 0), parity,
                          {p: v[M + half:] for p, v in sums.items() if v.shape[0] > M + half})
            for i in range(2):
                for n in range(_TILES):
                    y_part[1 - parity, i, n] = _collect(
                        i, n, {p: v[M:M + half] for p, v in sums.items()})
            return jnp.concatenate([_collect(parity, n, {p: v[:M] for p, v in sums.items()})
                                    for n in range(_TILES)], axis=1)

        chunk = STEP_UNROLL * seg

        def out_copy(start, n):
            return pltpu.make_async_copy(out_v.at[pl.ds(start, n)], out_hbm.at[pl.ds(start, n)],
                                         out_sem.at[0])

        def trip(it, mem):
            @pl.when(it == 1)
            def _():
                out_copy(0, chunk - seg).start()

            @pl.when(it > 1)
            def _():
                out_copy(pl.multiple_of((it - 1) * chunk - seg, seg), chunk).start()

            for u in range(STEP_UNROLL):
                mem = step(it * chunk + u * seg, u % 2, mem)
            return mem

        o_v[1] = jnp.zeros(o_v.shape[1:], F32)
        y_part[0] = jnp.zeros(y_part.shape[1:], F32)
        mem_cp.wait()
        n_trips = n_seg // STEP_UNROLL
        lax.fori_loop(0, n_trips, trip, mem_v[0].astype(F32))
        sent = (n_trips - 1) * chunk - seg
        out_copy(sent, chunk).start()
        late = {}
        for g in range(G + 1):
            before = tokens(o_v[1, :, _TILES * g * LANES:min(H, _TILES * (g + 1)) * LANES])
            for p in (_GROUP if g < G else _PAIR_OUT)[0]:
                d = _dot(_factor(p, 0, before), _as_bf16(wo_w[_slot(g, p)]))
                late[p] = d + late[p] if p in late else d
        finish_output(S - seg, 0, late)
        out_copy(S - seg, seg).start()
        out_copy(0, S).wait()

    pl.run_scoped(
        gmlp,
        pltpu.VMEM((2 * FH, D), BF16),
        pltpu.VMEM((S, S), BF16),
        pltpu.VMEM((8, LANES // 2, KD), U32),
        pltpu.VMEM((5, FH, KD), BF16),
        pltpu.VMEM((n_blocks, FH, LANES), F32),
        pltpu.VMEM((n_blocks, FH, LANES), F32),
        pltpu.VMEM((7, n_pairs, half_f, LANES), F32),
        pltpu.VMEM((2, 2, FH, LANES), F32),
        pltpu.VMEM((7, KF // LANES, half_d // 2, LANES), U32),
        pltpu.VMEM((D, FH - 2 * KF), BF16),
        pltpu.VMEM((FH, D), BF16),
        pltpu.VMEM((FH // CHUNK, 2, SUBLANES, LANES), F32),
        pltpu.VMEM((n_blocks, 2, LANES), F32),
        pltpu.VMEM((n_blocks, LANES), BF16),
        pltpu.VMEM((n_blocks, LANES), F32),
    )
    pl.run_scoped(
        recurrence,
        pltpu.VMEM((S, D), BF16),
        pltpu.VMEM((2, seg, H * LANES), F32),
        pltpu.VMEM((2, 2, _TILES, seg // 2, LANES), F32),
    )


@functools.partial(jax.jit, static_argnames=("A_seg_len",))
def pallas_recurrent_scan__memory_aug_recurrent_mem_tr__mixer_gmlp__prompt_kernel(
    A_x: jax.Array,
    A_mem0: jax.Array,
    A_Wq: jax.Array,
    A_Wk: jax.Array,
    A_Wv: jax.Array,
    A_Wo: jax.Array,
    A_seg_len: int,
    B_x: jax.Array,
    B_w_in: jax.Array,
    B_w_sp: jax.Array,
    B_b_sp: jax.Array,
    B_w_out: jax.Array,
):
    del B_x
    B, S, D = A_x.shape
    M = A_mem0.shape[1]
    _, H, Dh = A_Wq.shape
    F = B_w_in.shape[1]
    FH = F // 2
    seg = int(A_seg_len)
    assert B == 1 and Dh == LANES and D == _TILES * LANES and H % (2 * _TILES) == 2
    assert H // _TILES == 2 * (S // (4 * LANES) - 1)
    assert S % (2 * LANES) == 0 and S % (STEP_UNROLL * seg) == 0 and seg % (2 * SUBLANES) == 0
    KF = FH // (2 * LANES) * LANES

    assert KF // LANES == S // (4 * LANES) - 1

    n_groups = pl.cdiv(H, _TILES)
    n_factors = _slot(n_groups - 1, _PAIR_IN[2][-1]) + 1
    hbm = pl.BlockSpec(memory_space=pltpu.HBM)
    out = pl.pallas_call(
        functools.partial(_kernel, seg=seg),
        out_shape=jax.ShapeDtypeStruct((S, D), BF16),
        in_specs=[hbm] * 10,
        out_specs=hbm,
        scratch_shapes=[
            pltpu.VMEM((S, D), BF16),
            pltpu.VMEM((3, H // 2, D, LANES), U32),
            pltpu.VMEM((3, n_factors, LANES, LANES), BF16),
            pltpu.VMEM((n_factors, LANES, LANES), BF16),
            pltpu.VMEM((D // LANES, H * Dh, LANES), BF16),
            pltpu.VMEM((S, D), F32),
            pltpu.VMEM((S, D), F32),
            pltpu.VMEM((2, 3, n_groups, 2 * _TILES, seg // 2, LANES), F32),
            pltpu.VMEM((SUBLANES, M, D), BF16),
            pltpu.SemaphoreType.DMA((S // (2 * LANES),)),
            pltpu.SemaphoreType.DMA((FH // CHUNK,)),
            pltpu.SemaphoreType.DMA((S // (2 * LANES),)),
            pltpu.SemaphoreType.DMA((S // (4 * LANES),)),
            pltpu.SemaphoreType.DMA((5,)),
            pltpu.SemaphoreType.DMA((1,)),
        ],
        compiler_params=pltpu.CompilerParams(
            vmem_limit_bytes=VMEM_LIMIT),
    )(
        A_x.reshape(S, D),
        A_mem0.reshape(M, D),
        A_Wq,
        A_Wk,
        A_Wv,
        A_Wo.reshape(H * Dh, D),
        B_w_in.T,
        B_w_sp,
        B_b_sp.reshape(S // LANES, LANES),
        B_w_out,
    )
    return out.reshape(B, S, D)
```
